```python
import jax
import jax.numpy as jnp

def _softmax(x, axis=-1):
    return jax.nn.softmax(x, axis=axis)

def _gelu(x):
    return jax.nn.gelu(x, approximate=True)

def _silu(x):
    return jax.nn.silu(x)

def _sigmoid(x):
    return jax.nn.sigmoid(x)

def _layernorm(x, axis=-1, eps=1e-05):
    m = jnp.mean(x, axis=axis, keepdims=True)
    v = jnp.var(x, axis=axis, keepdims=True)
    return (x - m) / jnp.sqrt(v + eps)

def _scatter_add(tgt, idx, src, axis=0):
    return tgt.at[idx].add(src)

def _segment_sum(src, seg, n):
    return jax.ops.segment_sum(src, seg, n)

class _Rng:

    def __init__(self, key):
        self._k = key

    def _next(self):
        self._k, sub = jax.random.split(self._k)
        return sub

    def normal(self, shape):
        return jax.random.normal(self._next(), shape, dtype=jnp.bfloat16)

    def randint(self, lo, hi, shape):
        return jax.random.randint(self._next(), shape, lo, hi, dtype=jnp.int32)

    def uniform(self, shape, lo=0.0, hi=1.0):
        return jax.random.uniform(self._next(), shape, jnp.bfloat16, lo, hi)

    def permutation(self, n):
        return jax.random.permutation(self._next(), n)
kernel_name = 'standalone__dilated_atrous__vision'

def setup_inputs():
    _rng = _Rng(jax.random.key(int.from_bytes(__import__("os").urandom(4), "little")))
    _w = lambda a: (lambda t: t.astype(jnp.bfloat16) if jnp.issubdtype(t.dtype, jnp.floating) else t)(jnp.asarray(a))
    H = W = 384
    C = 384
    k = 1
    return {'x': _w((lambda *s: _rng.normal(s) * 0.05)(1, H, W, C)), 'w': _w((lambda *s: _rng.normal(s) * 0.05)(k, k, C, C) * (1.0 / (k * C ** 0.5)))}

def reference(x, w):
    B, H, W, C = x.shape
    k = 1
    rate = 2
    pad = (k - 1) * rate // 2
    xp = jnp.pad(x, ((0, 0), (pad, pad), (pad, pad), (0, 0)))
    out = jnp.zeros_like(x)
    for i in range(k):
        for j in range(k):
            tap = xp[:, i * rate:i * rate + H, j * rate:j * rate + W, :].copy()
            out = out + jnp.einsum('bhwc,co->bhwo', tap, w[i, j])
    return out
```

```python
import jax
import jax.numpy as jnp
from jax import lax
import jax.experimental.pallas as pl
import jax.experimental.pallas.tpu as pltpu

_SLAB = 4096
_PIECE = 64
_TM = 1024
_R_SLABS = 12
_R_SPLIT = 4
_R_COLS = 8
_R_TAIL = 32
_W_SLABS = 6
_W_COLS = 16
_W_RATE = (7, 8)


def _split(i, n):
    assert n & (n - 1) == 0
    if isinstance(i, int):
        return divmod(i, n)
    return lax.shift_right_logical(i, n.bit_length() - 1), i & (n - 1)


def _window(t, slabs, cols):
    group, j = _split(t, _SLAB // _PIECE // cols)
    start = j * (cols * _PIECE)
    if not isinstance(t, int):
        start = pl.multiple_of(start, cols * _PIECE)
    return group, (pl.ds(group * slabs, slabs), pl.ds(start, cols * _PIECE))


@jax.jit
def pallas_standalone__dilated_atrous__vision_kernel(
    x: jax.Array,
    w: jax.Array,
):
    B, H, W, C = x.shape
    assert w.shape == (1, 1, C, C) and C % 128 == 0
    M = B * H * W
    nc = C // 128
    n_slabs = M * nc // _SLAB
    n_steps = M // _TM
    assert n_slabs * _SLAB == M * nc and n_steps * _TM == M

    r_groups = n_slabs // _R_SLABS
    r_steps = n_steps // r_groups
    r_first = _SLAB // _PIECE // _R_COLS
    r_rounds = r_groups * r_first
    hops = _R_SLABS // _R_SPLIT
    r_copies = _R_COLS * hops
    last_read = r_rounds - 1 - r_first
    w_groups = n_slabs // _W_SLABS
    w_steps = n_steps // w_groups
    w_group_rounds = _SLAB // _PIECE // _W_COLS
    assert r_groups * _R_SLABS == n_slabs and r_groups * r_steps == n_steps
    assert w_groups * _W_SLABS == n_slabs and w_groups * w_steps == n_steps
    assert r_first <= r_steps and w_steps <= last_read <= n_steps - r_steps

    def kernel_function(x_hbm, w_hbm, o_hbm, buf, wbuf):
        def run(read_sems, w_sem, write_sem):
            def reader(t):
                group, window = _window(t, _R_SLABS, _R_COLS)
                src, dst = x_hbm.at[window], buf.at[window]

                def start(k, queue):
                    col, hop = divmod(k, hops)
                    slabs = (pl.ds(hop * _R_SPLIT, _R_SPLIT - 1) if queue
                             else pl.ds((hop + 1) * _R_SPLIT - 1, 1))
                    idx = (slabs, pl.ds(col * _PIECE, _PIECE))
                    pltpu.make_async_copy(
                        src.at[idx], dst.at[idx], read_sems.at[group]
                    ).start(priority=queue)

                return start

            def read_round(t, _=None):
                ahead, current = reader(t + 1), reader(t)
                for k in range(r_copies):
                    ahead(k, 1)
                    current(k, 0)

            def read_last_rounds(t):
                cols = r_copies - hops
                small = _R_SLABS * _PIECE // _R_TAIL
                final, current = reader(r_rounds - 1), reader(t)

                def ahead(k):
                    if k < cols:
                        return final(k, 1)
                    part, slab = divmod(k - cols, _R_SLABS)
                    idx = (n_slabs - _R_SLABS + slab,
                           pl.ds(_SLAB - _PIECE + part * _R_TAIL, _R_TAIL))
                    pltpu.make_async_copy(
                        x_hbm.at[idx], buf.at[idx], read_sems.at[r_groups - 1]
                    ).start(priority=1)

                if t == r_rounds - 2:
                    for k in range(r_copies):
                        ahead(k)
                        current(k, 0)
                    return
                for k in range(max(cols + small - r_copies, cols)):
                    if r_copies + k < cols + small:
                        ahead(r_copies + k)
                    if k < cols:
                        current(k, 0)

            def write_round(t, _=None):
                _, window = _window(t, _W_SLABS, _W_COLS)
                src, dst = buf.at[window], o_hbm.at[window]
                for col in range(_W_COLS):
                    idx = (slice(None), pl.ds(col * _PIECE, _PIECE))
                    pltpu.make_async_copy(src.at[idx], dst.at[idx], write_sem).start()

            def matmul(i):
                refs = []
                for n in range(nc):
                    slab, j = _split(nc * i + n, _SLAB // _TM)
                    refs.append(buf.at[slab, pl.ds(pl.multiple_of(j * _TM, _TM), _TM)])
                tiles = jnp.concatenate([r[...] for r in refs], axis=0)
                tiles = tiles.reshape(_TM // 8, nc, 8, 128)
                lhs = jnp.concatenate(
                    [tiles[:, n].reshape(_TM, 128) for n in range(nc)], axis=1)
                res = jnp.dot(lhs, wbuf[...], preferred_element_type=jnp.float32)
                tiles = jnp.stack(
                    [res[:, n * 128:(n + 1) * 128].reshape(_TM // 8, 8, 128)
                     for n in range(nc)], axis=1)
                lines = tiles.reshape(nc * _TM, 128).astype(buf.dtype)
                for n, r in enumerate(refs):
                    r[...] = lines[n * _TM:(n + 1) * _TM]

            w_copy = pltpu.make_async_copy(w_hbm, wbuf, w_sem)
            w_copy.start(priority=1)
            first = reader(0)
            for k in range(r_copies):
                first(k, 1)
            lax.fori_loop(0, r_first, read_round, None)
            w_copy.wait()

            def step(i, written):
                pl.when(i < last_read - 1)(lambda: read_round(r_first + i))
                pl.when(i == last_read - 1)(lambda: read_last_rounds(r_rounds - 2))

                @pl.when(i == last_read)
                def _():
                    read_last_rounds(r_rounds - 1)
                    write_round(0)

                computed = _split(i, w_steps)[0] * w_group_rounds
                due = 1 + _split(jnp.maximum(i - last_read, 0) * _W_RATE[0], _W_RATE[1])[0]
                write = jnp.minimum(computed, due) > written
                pl.when(write)(lambda: write_round(written))

                group, j = _split(i, r_steps)

                @pl.when(j == 0)
                def _():
                    slabs = pl.ds(group * _R_SLABS, _R_SLABS)
                    pltpu.make_async_copy(
                        x_hbm.at[slabs], buf.at[slabs], read_sems.at[group]).wait()

                matmul(i)
                return written + write.astype(jnp.int32)

            written = lax.fori_loop(0, n_steps, step, jnp.int32(1))
            lax.fori_loop(written, w_groups * w_group_rounds, write_round, None)
            pltpu.make_async_copy(buf, o_hbm, write_sem).wait()

        pl.run_scoped(
            run,
            pltpu.SemaphoreType.DMA((r_groups,)),
            pltpu.SemaphoreType.DMA(()),
            pltpu.SemaphoreType.DMA(()),
        )

    lines = x.reshape(M // 8, 8, nc, 128).transpose(0, 2, 1, 3)
    out = pl.pallas_call(
        kernel_function,
        in_specs=[
            pl.BlockSpec(memory_space=pl.ANY),
            pl.BlockSpec(memory_space=pl.ANY),
        ],
        out_specs=pl.BlockSpec(memory_space=pl.ANY),
        out_shape=jax.ShapeDtypeStruct((n_slabs, _SLAB, 128), x.dtype),
        scratch_shapes=[
            pltpu.VMEM((n_slabs, _SLAB, 128), x.dtype),
            pltpu.VMEM((C, C), w.dtype),
        ],
        compiler_params=pltpu.CompilerParams(
            vmem_limit_bytes=120 * 2**20, disable_bounds_checks=True),
    )(lines.reshape(n_slabs, _SLAB, 128), w.reshape(C, C))
    return out.reshape(M // 8, nc, 8, 128).transpose(0, 2, 1, 3).reshape(B, H, W, C)
```

```python
import jax
import jax.numpy as jnp
from jax import lax
import jax.experimental.pallas as pl
import jax.experimental.pallas.tpu as pltpu

_SLAB = 4096
_PIECE = 64
_TM = 1024
_R_SLABS = 12
_R_SPLIT = 4
_R_COLS = 8
_R_LEAD = 25
_R_TAIL = 5
_W_SLABS = 6
_W_COLS = 16
_W_RATE = (27, 32)


def _split(i, n):
    assert n & (n - 1) == 0
    if isinstance(i, int):
        return divmod(i, n)
    return lax.shift_right_logical(i, n.bit_length() - 1), i & (n - 1)


def _window(t, slabs, cols):
    group, j = _split(t, _SLAB // _PIECE // cols)
    start = j * (cols * _PIECE)
    if not isinstance(t, int):
        start = pl.multiple_of(start, cols * _PIECE)
    return group, (pl.ds(group * slabs, slabs), pl.ds(start, cols * _PIECE))


@jax.jit
def pallas_standalone__dilated_atrous__vision_kernel(
    x: jax.Array,
    w: jax.Array,
):
    B, H, W, C = x.shape
    assert w.shape == (1, 1, C, C) and C % 128 == 0
    M = B * H * W
    nc = C // 128
    n_slabs = M * nc // _SLAB
    n_steps = M // _TM
    assert n_slabs * _SLAB == M * nc and n_steps * _TM == M

    r_groups = n_slabs // _R_SLABS
    r_steps = n_steps // r_groups
    r_first = _SLAB // _PIECE // _R_COLS
    r_rounds = r_groups * r_first
    hops = _R_SLABS // _R_SPLIT
    r_copies = _R_COLS * hops
    r_whole = 2 * r_copies - _R_TAIL
    r_small = _R_TAIL * _R_SPLIT * _PIECE // 8
    last_read = r_rounds - 1 - r_first
    w_groups = n_slabs // _W_SLABS
    w_steps = n_steps // w_groups
    w_group_rounds = _SLAB // _PIECE // _W_COLS
    assert r_groups * _R_SLABS == n_slabs and r_groups * r_steps == n_steps
    assert w_groups * _W_SLABS == n_slabs and w_groups * w_steps == n_steps
    assert r_first <= r_steps and w_steps <= last_read <= n_steps - r_steps
    assert _R_LEAD <= min(r_whole, r_small)

    def kernel_function(x_hbm, w_hbm, o_hbm, buf, wbuf):
        def run(read_sems, w_sem, write_sem):
            def reader(t):
                views = {}

                def start(k, queue):
                    ahead, k = divmod(k, r_copies)
                    if ahead not in views:
                        group, window = _window(t + ahead, _R_SLABS, _R_COLS)
                        views[ahead] = (
                            x_hbm.at[window], buf.at[window], read_sems.at[group])
                    src, dst, sem = views[ahead]
                    col, hop = divmod(k, hops)
                    slabs = (pl.ds(hop * _R_SPLIT, _R_SPLIT - 1) if queue
                             else pl.ds((hop + 1) * _R_SPLIT - 1, 1))
                    idx = (slabs, pl.ds(col * _PIECE, _PIECE))
                    pltpu.make_async_copy(src.at[idx], dst.at[idx], sem).start(
                        priority=queue)

                return start

            def read_round(t, _=None):
                start = reader(t)
                for k in range(r_copies):
                    start(k + _R_LEAD, 1)
                    start(k, 0)

            def read_last_rounds(lo, hi):
                start = reader(r_rounds - 2)
                for k in range(lo, hi):
                    piece, tile = divmod(k + _R_LEAD - r_whole, _PIECE // 8)
                    if piece < 0:
                        start(k + _R_LEAD, 1)
                    else:
                        col, slab = divmod(piece - _R_TAIL * _R_SPLIT, _R_SLABS)
                        idx = (n_slabs - _R_SLABS + slab,
                               pl.ds(_SLAB + col * _PIECE + tile * 8, 8))
                        pltpu.make_async_copy(
                            x_hbm.at[idx], buf.at[idx], read_sems.at[r_groups - 1]
                        ).start(priority=1)
                    if k < r_whole:
                        start(k, 0)

            def write_round(t, _=None):
                _, window = _window(t, _W_SLABS, _W_COLS)
                src, dst = buf.at[window], o_hbm.at[window]
                for col in range(_W_COLS):
                    idx = (slice(None), pl.ds(col * _PIECE, _PIECE))
                    pltpu.make_async_copy(src.at[idx], dst.at[idx], write_sem).start()

            def matmul(i):
                refs = []
                for n in range(nc):
                    slab, j = _split(nc * i + n, _SLAB // _TM)
                    refs.append(buf.at[slab, pl.ds(pl.multiple_of(j * _TM, _TM), _TM)])
                tiles = jnp.concatenate([r[...] for r in refs], axis=0)
                tiles = tiles.reshape(_TM // 8, nc, 8, 128)
                lhs = jnp.concatenate(
                    [tiles[:, n].reshape(_TM, 128) for n in range(nc)], axis=1)
                res = jnp.dot(lhs, wbuf[...], preferred_element_type=jnp.float32)
                tiles = jnp.stack(
                    [res[:, n * 128:(n + 1) * 128].reshape(_TM // 8, 8, 128)
                     for n in range(nc)], axis=1)
                lines = tiles.reshape(nc * _TM, 128).astype(buf.dtype)
                for n, r in enumerate(refs):
                    r[...] = lines[n * _TM:(n + 1) * _TM]

            w_copy = pltpu.make_async_copy(w_hbm, wbuf, w_sem)
            w_copy.start(priority=1)
            first = reader(0)
            for k in range(_R_LEAD):
                first(k, 1)
            lax.fori_loop(0, r_first, read_round, None)
            w_copy.wait()

            def step(i, written):
                pl.when(i < last_read - 1)(lambda: read_round(r_first + i))
                pl.when(i == last_read - 1)(lambda: read_last_rounds(0, r_copies))

                @pl.when(i == last_read)
                def _():
                    read_last_rounds(r_copies, r_whole + r_small - _R_LEAD)
                    write_round(0)

                computed = _split(i, w_steps)[0] * w_group_rounds
                steps = jnp.maximum(i - last_read, 0) + 1
                due = 1 + _split(steps * _W_RATE[0], _W_RATE[1])[0]
                write = jnp.minimum(computed, due) > written
                pl.when(write)(lambda: write_round(written))

                group, j = _split(i, r_steps)

                @pl.when(j == 0)
                def _():
                    slabs = pl.ds(group * _R_SLABS, _R_SLABS)
                    pltpu.make_async_copy(
                        x_hbm.at[slabs], buf.at[slabs], read_sems.at[group]).wait()

                matmul(i)
                return written + write.astype(jnp.int32)

            written = lax.fori_loop(0, n_steps, step, jnp.int32(1))
            lax.fori_loop(written, w_groups * w_group_rounds, write_round, None)
            pltpu.make_async_copy(buf, o_hbm, write_sem).wait()

        pl.run_scoped(
            run,
            pltpu.SemaphoreType.DMA((r_groups,)),
            pltpu.SemaphoreType.DMA(()),
            pltpu.SemaphoreType.DMA(()),
        )

    lines = x.reshape(M // 8, 8, nc, 128).transpose(0, 2, 1, 3)
    out = pl.pallas_call(
        kernel_function,
        in_specs=[
            pl.BlockSpec(memory_space=pl.ANY),
            pl.BlockSpec(memory_space=pl.ANY),
        ],
        out_specs=pl.BlockSpec(memory_space=pl.ANY),
        out_shape=jax.ShapeDtypeStruct((n_slabs, _SLAB, 128), x.dtype),
        scratch_shapes=[
            pltpu.VMEM((n_slabs, _SLAB, 128), x.dtype),
            pltpu.VMEM((C, C), w.dtype),
        ],
        compiler_params=pltpu.CompilerParams(
            vmem_limit_bytes=120 * 2**20, disable_bounds_checks=True),
    )(lines.reshape(n_slabs, _SLAB, 128), w.reshape(C, C))
    return out.reshape(M // 8, nc, 8, 128).transpose(0, 2, 1, 3).reshape(B, H, W, C)
```

```python
import jax
import jax.numpy as jnp
from jax import lax
import jax.experimental.pallas as pl
import jax.experimental.pallas.tpu as pltpu

_SLAB = 4096
_PIECE = 64
_TM = 1024
_R_SLABS = 12
_R_SPLIT = 4
_R_COLS = 8
_R_LEAD = 26
_R_TAIL = 8
_W_SLABS = 6
_W_COLS = 16
_W_RATE = (27, 32)


def _split(i, n):
    assert n & (n - 1) == 0
    if isinstance(i, int):
        return divmod(i, n)
    return lax.shift_right_logical(i, n.bit_length() - 1), i & (n - 1)


def _window(t, slabs, cols):
    group, j = _split(t, _SLAB // _PIECE // cols)
    start = j * (cols * _PIECE)
    if not isinstance(t, int):
        start = pl.multiple_of(start, cols * _PIECE)
    return group, (pl.ds(group * slabs, slabs), pl.ds(start, cols * _PIECE))


@jax.jit
def pallas_standalone__dilated_atrous__vision_kernel(
    x: jax.Array,
    w: jax.Array,
):
    B, H, W, C = x.shape
    assert w.shape == (1, 1, C, C) and C % 128 == 0
    M = B * H * W
    nc = C // 128
    n_slabs = M * nc // _SLAB
    n_steps = M // _TM
    assert n_slabs * _SLAB == M * nc and n_steps * _TM == M

    r_groups = n_slabs // _R_SLABS
    r_steps = n_steps // r_groups
    r_first = _SLAB // _PIECE // _R_COLS
    r_rounds = r_groups * r_first
    hops = _R_SLABS // _R_SPLIT
    r_copies = _R_COLS * hops
    r_whole = 2 * r_copies - 1
    r_small = _R_SPLIT * _PIECE // _R_TAIL
    last_read = r_rounds - 1 - r_first
    w_groups = n_slabs // _W_SLABS
    w_steps = n_steps // w_groups
    w_group_rounds = _SLAB // _PIECE // _W_COLS
    assert r_groups * _R_SLABS == n_slabs and r_groups * r_steps == n_steps
    assert w_groups * _W_SLABS == n_slabs and w_groups * w_steps == n_steps
    assert r_first <= r_steps and w_steps <= last_read <= n_steps - r_steps
    assert _R_LEAD <= min(r_whole, r_small)

    def kernel_function(x_hbm, w_hbm, o_hbm, buf, wbuf):
        def run(read_sems, w_sem, write_sem):
            def reader(t):
                views = {}

                def start(k, queue):
                    ahead, k = divmod(k, r_copies)
                    if ahead not in views:
                        group, window = _window(t + ahead, _R_SLABS, _R_COLS)
                        views[ahead] = (
                            x_hbm.at[window], buf.at[window], read_sems.at[group])
                    src, dst, sem = views[ahead]
                    col, hop = divmod(k, hops)
                    slabs = (pl.ds(hop * _R_SPLIT, _R_SPLIT - 1) if queue
                             else pl.ds((hop + 1) * _R_SPLIT - 1, 1))
                    idx = (slabs, pl.ds(col * _PIECE, _PIECE))
                    pltpu.make_async_copy(src.at[idx], dst.at[idx], sem).start(
                        priority=queue)

                return start

            def read_round(t, _=None):
                start = reader(t)
                for k in range(r_copies):
                    start(k + _R_LEAD, 1)
                    start(k, 0)

            def read_last_rounds(lo, hi):
                start = reader(r_rounds - 2)
                for k in range(lo, hi):
                    slab, part = divmod(k + _R_LEAD - r_whole, _PIECE // _R_TAIL)
                    if slab < 0:
                        start(k + _R_LEAD, 1)
                    else:
                        idx = (n_slabs - _R_SPLIT + slab,
                               pl.ds(_SLAB - _PIECE + part * _R_TAIL, _R_TAIL))
                        pltpu.make_async_copy(
                            x_hbm.at[idx], buf.at[idx], read_sems.at[r_groups - 1]
                        ).start(priority=1)
                    if k < r_whole:
                        start(k, 0)

            def write_round(t, _=None):
                _, window = _window(t, _W_SLABS, _W_COLS)
                src, dst = buf.at[window], o_hbm.at[window]
                for col in range(_W_COLS):
                    idx = (slice(None), pl.ds(col * _PIECE, _PIECE))
                    pltpu.make_async_copy(src.at[idx], dst.at[idx], write_sem).start()

            def matmul(i):
                refs = []
                for n in range(nc):
                    slab, j = _split(nc * i + n, _SLAB // _TM)
                    refs.append(buf.at[slab, pl.ds(pl.multiple_of(j * _TM, _TM), _TM)])
                tiles = jnp.concatenate([r[...] for r in refs], axis=0)
                tiles = tiles.reshape(_TM // 8, nc, 8, 128)
                lhs = jnp.concatenate(
                    [tiles[:, n].reshape(_TM, 128) for n in range(nc)], axis=1)
                res = jnp.dot(lhs, wbuf[...], preferred_element_type=jnp.float32)
                tiles = jnp.stack(
                    [res[:, n * 128:(n + 1) * 128].reshape(_TM // 8, 8, 128)
                     for n in range(nc)], axis=1)
                lines = tiles.reshape(nc * _TM, 128).astype(buf.dtype)
                for n, r in enumerate(refs):
                    r[...] = lines[n * _TM:(n + 1) * _TM]

            w_copy = pltpu.make_async_copy(w_hbm, wbuf, w_sem)
            w_copy.start(priority=1)
            first = reader(0)
            for k in range(_R_LEAD):
                first(k, 1)
            lax.fori_loop(0, r_first, read_round, None)
            w_copy.wait()

            def step(i, written):
                pl.when(i < last_read - 1)(lambda: read_round(r_first + i))
                pl.when(i == last_read - 1)(lambda: read_last_rounds(0, r_copies))

                @pl.when(i == last_read)
                def _():
                    read_last_rounds(r_copies, r_whole + r_small - _R_LEAD)
                    write_round(0)

                computed = _split(i, w_steps)[0] * w_group_rounds
                steps = jnp.maximum(i - last_read, 0) + 1
                due = 1 + _split(steps * _W_RATE[0], _W_RATE[1])[0]
                write = jnp.minimum(computed, due) > written
                pl.when(write)(lambda: write_round(written))

                group, j = _split(i, r_steps)

                @pl.when(j == 0)
                def _():
                    slabs = pl.ds(group * _R_SLABS, _R_SLABS)
                    pltpu.make_async_copy(
                        x_hbm.at[slabs], buf.at[slabs], read_sems.at[group]).wait()

                matmul(i)
                return written + write.astype(jnp.int32)

            written = lax.fori_loop(0, n_steps, step, jnp.int32(1))
            lax.fori_loop(written, w_groups * w_group_rounds, write_round, None)
            pltpu.make_async_copy(buf, o_hbm, write_sem).wait()

        pl.run_scoped(
            run,
            pltpu.SemaphoreType.DMA((r_groups,)),
            pltpu.SemaphoreType.DMA(()),
            pltpu.SemaphoreType.DMA(()),
        )

    lines = x.reshape(M // 8, 8, nc, 128).transpose(0, 2, 1, 3)
    out = pl.pallas_call(
        kernel_function,
        in_specs=[
            pl.BlockSpec(memory_space=pl.ANY),
            pl.BlockSpec(memory_space=pl.ANY),
        ],
        out_specs=pl.BlockSpec(memory_space=pl.ANY),
        out_shape=jax.ShapeDtypeStruct((n_slabs, _SLAB, 128), x.dtype),
        scratch_shapes=[
            pltpu.VMEM((n_slabs, _SLAB, 128), x.dtype),
            pltpu.VMEM((C, C), w.dtype),
        ],
        compiler_params=pltpu.CompilerParams(
            vmem_limit_bytes=120 * 2**20, disable_bounds_checks=True),
    )(lines.reshape(n_slabs, _SLAB, 128), w.reshape(C, C))
    return out.reshape(M // 8, nc, 8, 128).transpose(0, 2, 1, 3).reshape(B, H, W, C)
```

```python
import jax
import jax.numpy as jnp
from jax import lax
import jax.experimental.pallas as pl
import jax.experimental.pallas.tpu as pltpu

_SLAB = 4096
_PIECE = 64
_TM = 1024
_R_SLABS = 12
_R_SPLIT = 4
_R_COLS = 8
_R_LEAD = 25
_R_TAIL = 2
_SMALL = 16
_W_SLABS = 6
_W_COLS = 16
_W_RATE = (27, 32)


def _split(i, n):
    assert n & (n - 1) == 0
    if isinstance(i, int):
        return divmod(i, n)
    return lax.shift_right_logical(i, n.bit_length() - 1), i & (n - 1)


def _window(t, slabs, cols):
    group, j = _split(t, _SLAB // _PIECE // cols)
    start = j * (cols * _PIECE)
    if not isinstance(t, int):
        start = pl.multiple_of(start, cols * _PIECE)
    return group, (pl.ds(group * slabs, slabs), pl.ds(start, cols * _PIECE))


@jax.jit
def pallas_standalone__dilated_atrous__vision_kernel(
    x: jax.Array,
    w: jax.Array,
):
    B, H, W, C = x.shape
    assert w.shape == (1, 1, C, C) and C % 128 == 0
    M = B * H * W
    nc = C // 128
    n_slabs = M * nc // _SLAB
    n_steps = M // _TM
    assert n_slabs * _SLAB == M * nc and n_steps * _TM == M

    r_groups = n_slabs // _R_SLABS
    r_steps = n_steps // r_groups
    r_first = _SLAB // _PIECE // _R_COLS
    r_rounds = r_groups * r_first
    hops = _R_SLABS // _R_SPLIT
    r_copies = _R_COLS * hops
    r_whole = 2 * r_copies - _R_TAIL
    r_small = _R_TAIL * _R_SPLIT * _PIECE // _SMALL
    last_read = r_rounds - 1 - r_first
    w_groups = n_slabs // _W_SLABS
    w_steps = n_steps // w_groups
    w_group_rounds = _SLAB // _PIECE // _W_COLS
    assert r_groups * _R_SLABS == n_slabs and r_groups * r_steps == n_steps
    assert w_groups * _W_SLABS == n_slabs and w_groups * w_steps == n_steps
    assert r_first <= r_steps and w_steps <= last_read <= n_steps - r_steps
    assert _R_LEAD <= min(r_whole, r_small)

    def kernel_function(x_hbm, w_hbm, o_hbm, buf, wbuf):
        def run(read_sems, w_sem, write_sem):
            def reader(t):
                views = {}

                def start(k, queue):
                    ahead, k = divmod(k, r_copies)
                    if ahead not in views:
                        group, window = _window(t + ahead, _R_SLABS, _R_COLS)
                        views[ahead] = (
                            x_hbm.at[window], buf.at[window], read_sems.at[group])
                    src, dst, sem = views[ahead]
                    col, hop = divmod(k, hops)
                    slabs = (pl.ds(hop * _R_SPLIT, _R_SPLIT - 1) if queue
                             else pl.ds((hop + 1) * _R_SPLIT - 1, 1))
                    idx = (slabs, pl.ds(col * _PIECE, _PIECE))
                    pltpu.make_async_copy(src.at[idx], dst.at[idx], sem).start(
                        priority=queue)

                return start

            def read_round(t, _=None):
                start = reader(t)
                for k in range(r_copies):
                    start(k + _R_LEAD, 1)
                    start(k, 0)

            def read_last_rounds(lo, hi):
                start = reader(r_rounds - 2)
                for k in range(lo, hi):
                    piece, part = divmod(k + _R_LEAD - r_whole, _PIECE // _SMALL)
                    if piece < 0:
                        start(k + _R_LEAD, 1)
                    else:
                        col, slab = divmod(piece - _R_TAIL * _R_SPLIT, _R_SLABS)
                        idx = (n_slabs - _R_SLABS + slab,
                               pl.ds(_SLAB + col * _PIECE + part * _SMALL, _SMALL))
                        pltpu.make_async_copy(
                            x_hbm.at[idx], buf.at[idx], read_sems.at[r_groups - 1]
                        ).start(priority=1)
                    if k < r_whole:
                        start(k, 0)

            def write_round(t, _=None):
                _, window = _window(t, _W_SLABS, _W_COLS)
                src, dst = buf.at[window], o_hbm.at[window]
                for col in range(_W_COLS):
                    idx = (slice(None), pl.ds(col * _PIECE, _PIECE))
                    pltpu.make_async_copy(src.at[idx], dst.at[idx], write_sem).start()

            def matmul(i):
                refs = []
                for n in range(nc):
                    slab, j = _split(nc * i + n, _SLAB // _TM)
                    refs.append(buf.at[slab, pl.ds(pl.multiple_of(j * _TM, _TM), _TM)])
                tiles = jnp.concatenate([r[...] for r in refs], axis=0)
                tiles = tiles.reshape(_TM // 8, nc, 8, 128)
                lhs = jnp.concatenate(
                    [tiles[:, n].reshape(_TM, 128) for n in range(nc)], axis=1)
                res = jnp.dot(lhs, wbuf[...], preferred_element_type=jnp.float32)
                tiles = jnp.stack(
                    [res[:, n * 128:(n + 1) * 128].reshape(_TM // 8, 8, 128)
                     for n in range(nc)], axis=1)
                lines = tiles.reshape(nc * _TM, 128).astype(buf.dtype)
                for n, r in enumerate(refs):
                    r[...] = lines[n * _TM:(n + 1) * _TM]

            w_copy = pltpu.make_async_copy(w_hbm, wbuf, w_sem)
            w_copy.start(priority=1)
            first = reader(0)
            for k in range(_R_LEAD):
                first(k, 1)
            lax.fori_loop(0, r_first, read_round, None)
            w_copy.wait()

            def step(i, written):
                pl.when(i < last_read - 1)(lambda: read_round(r_first + i))
                pl.when(i == last_read - 1)(lambda: read_last_rounds(0, r_copies))

                @pl.when(i == last_read)
                def _():
                    read_last_rounds(r_copies, r_whole + r_small - _R_LEAD)
                    write_round(0)

                computed = _split(i, w_steps)[0] * w_group_rounds
                steps = jnp.maximum(i - last_read, 0) + 1
                due = 1 + _split(steps * _W_RATE[0], _W_RATE[1])[0]
                write = jnp.minimum(computed, due) > written
                pl.when(write)(lambda: write_round(written))

                group, j = _split(i, r_steps)

                @pl.when(j == 0)
                def _():
                    slabs = pl.ds(group * _R_SLABS, _R_SLABS)
                    pltpu.make_async_copy(
                        x_hbm.at[slabs], buf.at[slabs], read_sems.at[group]).wait()

                matmul(i)
                return written + write.astype(jnp.int32)

            written = lax.fori_loop(0, n_steps, step, jnp.int32(1))
            lax.fori_loop(written, w_groups * w_group_rounds, write_round, None)
            pltpu.make_async_copy(buf, o_hbm, write_sem).wait()

        pl.run_scoped(
            run,
            pltpu.SemaphoreType.DMA((r_groups,)),
            pltpu.SemaphoreType.DMA(()),
            pltpu.SemaphoreType.DMA(()),
        )

    lines = x.reshape(M // 8, 8, nc, 128).transpose(0, 2, 1, 3)
    out = pl.pallas_call(
        kernel_function,
        in_specs=[
            pl.BlockSpec(memory_space=pl.ANY),
            pl.BlockSpec(memory_space=pl.ANY),
        ],
        out_specs=pl.BlockSpec(memory_space=pl.ANY),
        out_shape=jax.ShapeDtypeStruct((n_slabs, _SLAB, 128), x.dtype),
        scratch_shapes=[
            pltpu.VMEM((n_slabs, _SLAB, 128), x.dtype),
            pltpu.VMEM((C, C), w.dtype),
        ],
        compiler_params=pltpu.CompilerParams(
            vmem_limit_bytes=120 * 2**20, disable_bounds_checks=True),
    )(lines.reshape(n_slabs, _SLAB, 128), w.reshape(C, C))
    return out.reshape(M // 8, nc, 8, 128).transpose(0, 2, 1, 3).reshape(B, H, W, C)
```
